```python
import jax
import jax.numpy as jnp

def _softmax(x, axis=-1):
    return jax.nn.softmax(x, axis=axis)
def _gelu(x):
    return jax.nn.gelu(x, approximate=True)
def _silu(x):
    return jax.nn.silu(x)
def _sigmoid(x):
    return jax.nn.sigmoid(x)
def _layernorm(x, axis=-1, eps=1e-5):
    m = jnp.mean(x, axis=axis, keepdims=True)
    v = jnp.var(x, axis=axis, keepdims=True)
    return (x - m) / jnp.sqrt(v + eps)
def _scatter_add(tgt, idx, src, axis=0):
    return tgt.at[idx].add(src)
def _segment_sum(src, seg, n):
    return jax.ops.segment_sum(src, seg, n)
class _Rng:
    def __init__(self, key):
        self._k = key
    def _next(self):
        self._k, sub = jax.random.split(self._k)
        return sub
    def normal(self, shape):
        return jax.random.normal(self._next(), shape, dtype=jnp.bfloat16)
    def randint(self, lo, hi, shape):
        return jax.random.randint(self._next(), shape, lo, hi, dtype=jnp.int32)
    def uniform(self, shape, lo=0.0, hi=1.0):
        return jax.random.uniform(self._next(), shape, jnp.bfloat16, lo, hi)
    def permutation(self, n):
        return jax.random.permutation(self._next(), n)


kernel_name = 'sequential_preLN__sliding_block_cached__mixer_s_mlp__decode'

def setup_inputs():
    _rng = _Rng(jax.random.key(int.from_bytes(__import__("os").urandom(4), "little")))
    _w = (lambda a: (lambda t: t.astype(jnp.bfloat16) if jnp.issubdtype(t.dtype, jnp.floating) else t)(jnp.asarray(a)))
    def _A_setup():
        B, Sq, D = 1, 1, 640
        Hq, Hkv, Sk, Dh = 32, 32, 32768, 192
        assert Hq % Hkv == 0, (Hq, Hkv)
        return {
            "x": _w((lambda *s: _rng.normal(s) * 0.05)(B, Sq, D)),
            "k_cache": _w((lambda *s: _rng.normal(s) * 0.05)(B, Hkv, Sk, Dh)),
            "v_cache": _w((lambda *s: _rng.normal(s) * 0.05)(B, Hkv, Sk, Dh)),
            "wq": _w((lambda *s: _rng.normal(s) * 0.05)(D, Hq * Dh) * (D ** -0.5)),
            "wo": _w((lambda *s: _rng.normal(s) * 0.05)(Hq * Dh, D) * ((Hq * Dh) ** -0.5)),
        }
    _A_in = _A_setup()

    def _B_setup():
        B, S, D, F = 1, 1, 640, 1536
        return {
            "x":  _w((lambda *s: _rng.normal(s) * 0.05)(B, S, D)),
            "w1": _w((lambda *s: _rng.normal(s) * 0.05)(D, D) * (D ** -0.5)),
            "w2": _w((lambda *s: _rng.normal(s) * 0.05)(D, D) * (D ** -0.5)),
            "w3": _w((lambda *s: _rng.normal(s) * 0.05)(D, F) * (D ** -0.5)),
            "w4": _w((lambda *s: _rng.normal(s) * 0.05)(F, D) * (F ** -0.5)),
        }
    _B_in = _B_setup()

    return {
        "A_x": _A_in["x"],
        "A_k_cache": _A_in["k_cache"],
        "A_v_cache": _A_in["v_cache"],
        "A_wq": _A_in["wq"],
        "A_wo": _A_in["wo"],
        "B_x": _B_in["x"],
        "B_w1": _B_in["w1"],
        "B_w2": _B_in["w2"],
        "B_w3": _B_in["w3"],
        "B_w4": _B_in["w4"],
    }

def reference(A_x, A_k_cache, A_v_cache, A_wq, A_wo, B_x, B_w1, B_w2, B_w3, B_w4):
    def _A_ref(x, k_cache, v_cache, wq, wo):
        B, Sq, D = x.shape
        Hq, Dh = 32, 192
        Hkv, Sk = k_cache.shape[1], k_cache.shape[2]
        W = min(4096, max(256, Sk // 4))
        rep = Hq // Hkv
        q = (lambda x, *d: x.transpose(*d))((x @ wq).reshape(B, Sq, Hq, Dh), 0, 2, 1, 3)
        k = jnp.repeat(k_cache[:, :, Sk - W:, :], rep, axis=1)
        v = jnp.repeat(v_cache[:, :, Sk - W:, :], rep, axis=1)
        scores = jnp.einsum("bhqd,bhkd->bhqk", q, k) * (Dh ** -0.5)
        p = _softmax(scores, axis=-1)
        o = jnp.einsum("bhqk,bhkd->bhqd", p, v)
        return (lambda x, *d: x.transpose(*d))(o, 0, 2, 1, 3).reshape(B, Sq, Hq * Dh) @ wo

    def _B_ref(x, w1, w2, w3, w4):
        B, S, D = x.shape
        h = _gelu(_layernorm(x, axis=-1) @ w1)
        c = D // 4
        g0 = jnp.pad(h[:, :, 0*c:1*c], ((0, 0), (1, 0), (0, 0)))[:, :S, :]
        g1 = jnp.pad(h[:, :, 1*c:2*c], ((0, 0), (0, 1), (0, 0)))[:, 1:, :]
        g2 = jnp.pad(h[:, :, 2*c:3*c], ((0, 0), (2, 0), (0, 0)))[:, :S, :]
        g3 = jnp.pad(h[:, :, 3*c:   ], ((0, 0), (0, 2), (0, 0)))[:, 2:, :]
        hs = jnp.concatenate([g0, g1, g2, g3], axis=-1) @ w2
        x1 = x + hs
        h2 = _gelu(_layernorm(x1, axis=-1) @ w3) @ w4
        return x1 + h2

    x = A_x
    h = x + _A_ref(_layernorm(x, axis=-1), A_k_cache, A_v_cache, A_wq, A_wo)
    h2 = h + _B_ref(_layernorm(h, axis=-1), B_w1, B_w2, B_w3, B_w4)
    return h2
```

```python
import functools

import jax
import jax.numpy as jnp
from jax import lax
import jax.experimental.pallas as pl
import jax.experimental.pallas.tpu as pltpu

_EPS = 1e-5
_F32 = jnp.float32
_BF16 = jnp.bfloat16


def _layernorm(x):
    m = jnp.mean(x, axis=-1, keepdims=True)
    c = x - m
    v = jnp.mean(c * c, axis=-1, keepdims=True)
    return c * lax.rsqrt(v + _EPS)


def _kernel(x_hbm, k_hbm, v_hbm, wq_hbm, wo_hbm, w3_hbm, w4_hbm,
            o_ref,
            xbuf, kbuf, vbuf, wqbuf, wobuf, w3buf, w4buf, qbuf,
            ksem, vsem, wsem,
            *, H, DH, SK, W, D, F, NBUF, NWQ, NW4):
    w0 = SK - W
    PAIR = 2 * DH
    wq_cols = (H * DH) // NWQ
    w4_rows = F // NW4

    def k_copy(h, slot):
        return pltpu.make_async_copy(
            k_hbm.at[0, h, :, pl.ds(w0, W)], kbuf.at[slot], ksem.at[slot])

    def v_copy(h, slot):
        return pltpu.make_async_copy(
            v_hbm.at[0, h, :, pl.ds(w0, W)], vbuf.at[slot], vsem.at[slot])

    x_copy = pltpu.make_async_copy(x_hbm, xbuf, wsem.at[0])
    wq_copies = [
        pltpu.make_async_copy(wq_hbm.at[:, pl.ds(i * wq_cols, wq_cols)],
                              wqbuf.at[:, pl.ds(i * wq_cols, wq_cols)],
                              wsem.at[1 + i]) for i in range(NWQ)]
    wo_copy = pltpu.make_async_copy(wo_hbm, wobuf, wsem.at[1 + NWQ])
    w3_copy = pltpu.make_async_copy(w3_hbm, w3buf, wsem.at[2 + NWQ])
    w4_copies = [
        pltpu.make_async_copy(w4_hbm.at[pl.ds(i * w4_rows, w4_rows), :],
                              w4buf.at[pl.ds(i * w4_rows, w4_rows), :],
                              wsem.at[3 + NWQ + i]) for i in range(NW4)]

    x_copy.start()
    for c in wq_copies:
        c.start()
    wo_copy.start()
    for h in range(NBUF):
        k_copy(h, h).start()
        v_copy(h, h).start()

    x_copy.wait()
    x = xbuf[0].astype(_F32)
    xn = _layernorm(x).astype(_BF16)
    xn8 = jnp.broadcast_to(xn, (8, D))
    scale = DH ** -0.5
    for i in range(NWQ):
        wq_copies[i].wait()
        q = jnp.dot(xn8, wqbuf[:, pl.ds(i * wq_cols, wq_cols)],
                    preferred_element_type=_F32)
        for j in range(wq_cols // DH):
            qbuf[i * (wq_cols // DH) + j] = q[:, j * DH:(j + 1) * DH].astype(_BF16)
    wo_copy.wait()

    def head(h, acc):
        slot = lax.rem(h, NBUF)
        k_copy(h, slot).wait()
        s = jnp.dot(qbuf[h], kbuf[slot], preferred_element_type=_F32) * scale
        m = jnp.max(s, axis=-1, keepdims=True)
        p = jnp.exp(s - m)
        l = jnp.sum(p, axis=-1, keepdims=True)

        @pl.when(h + NBUF < H)
        def _():
            k_copy(h + NBUF, slot).start()

        v_copy(h, slot).wait()
        o = lax.dot_general(p.astype(_BF16), vbuf[slot], (((1,), (1,)), ((), ())),
                            preferred_element_type=_F32)
        o = (o / l).astype(_BF16)

        @pl.when(h + NBUF < H)
        def _():
            v_copy(h + NBUF, slot).start()

        @pl.when(h + NBUF == H)
        def _():
            w3_copy.start()
            for c in w4_copies:
                c.start()

        wo_h = wobuf[pl.ds(pl.multiple_of(h * DH, 64), DH), :]
        return acc + jnp.dot(o, wo_h, preferred_element_type=_F32)

    attn = lax.fori_loop(0, H, head, jnp.zeros((8, D), _F32))

    h1 = x + attn[0:1]
    y = _layernorm(h1)
    z = _layernorm(y).astype(_BF16)
    z8 = jnp.broadcast_to(z, (8, D))
    w3_copy.wait()
    g = jax.nn.gelu(jnp.dot(z8, w3buf[...], preferred_element_type=_F32),
                    approximate=True).astype(_BF16)
    out = h1 + y
    for i in range(NW4):
        w4_copies[i].wait()
        out = out + jnp.dot(g[:, i * w4_rows:(i + 1) * w4_rows],
                            w4buf[pl.ds(i * w4_rows, w4_rows), :],
                            preferred_element_type=_F32)[0:1]
    o_ref[0] = out.astype(o_ref.dtype)


@jax.jit
def pallas_sequential_preLN__sliding_block_cached__mixer_s_mlp__decode_kernel(
    A_x: jax.Array,
    A_k_cache: jax.Array,
    A_v_cache: jax.Array,
    A_wq: jax.Array,
    A_wo: jax.Array,
    B_x: jax.Array,
    B_w1: jax.Array,
    B_w2: jax.Array,
    B_w3: jax.Array,
    B_w4: jax.Array,
):
    B, S, D = A_x.shape
    _, H, SK, DH = A_k_cache.shape
    F = B_w3.shape[1]
    assert B == 1 and S == 1
    W = min(4096, max(256, SK // 4))
    NBUF, NWQ, NW4 = 3, 4, 4

    kt = jnp.swapaxes(A_k_cache, 2, 3)
    vt = jnp.swapaxes(A_v_cache, 2, 3)

    kern = functools.partial(_kernel, H=H, DH=DH, SK=SK, W=W, D=D, F=F,
                             NBUF=NBUF, NWQ=NWQ, NW4=NW4)
    any_spec = pl.BlockSpec(memory_space=pl.ANY)
    return pl.pallas_call(
        kern,
        out_shape=jax.ShapeDtypeStruct((B, S, D), A_x.dtype),
        in_specs=[any_spec] * 7,
        out_specs=pl.BlockSpec(memory_space=pltpu.VMEM),
        scratch_shapes=[
            pltpu.VMEM((B, S, D), _BF16),
            pltpu.VMEM((NBUF, DH, W), _BF16),
            pltpu.VMEM((NBUF, DH, W), _BF16),
            pltpu.VMEM((D, H * DH), _BF16),
            pltpu.VMEM((H * DH, D), _BF16),
            pltpu.VMEM((D, F), _BF16),
            pltpu.VMEM((F, D), _BF16),
            pltpu.VMEM((H, 8, DH), _BF16),
            pltpu.SemaphoreType.DMA((NBUF,)),
            pltpu.SemaphoreType.DMA((NBUF,)),
            pltpu.SemaphoreType.DMA((3 + NWQ + NW4,)),
        ],
        compiler_params=pltpu.CompilerParams(vmem_limit_bytes=64 * 1024 * 1024),
    )(A_x, kt, vt, A_wq, A_wo, B_w3, B_w4)
```

```python
import functools

import jax
import jax.numpy as jnp
from jax import lax
import jax.experimental.pallas as pl
import jax.experimental.pallas.tpu as pltpu

_EPS = 1e-5
_F32 = jnp.float32
_BF16 = jnp.bfloat16

CFG = dict(COMPUTE=True, C=128, NW4=12, NPAIR=16, NR=64, LA=40, ORDER="10", MIX=False,
           WQR=8, WOR=8)


def _layernorm(x):
    m = jnp.mean(x, axis=-1, keepdims=True)
    c = x - m
    v = jnp.mean(c * c, axis=-1, keepdims=True)
    return c * lax.rsqrt(v + _EPS)


def _kernel(x_hbm, k_hbm, v_hbm, wq_hbm, wo_hbm, w3_hbm, w4_hbm,
            o_ref,
            xbuf, ring, wqbuf, wobuf, w3buf, w4buf, qbbuf, sbuf, accbuf,
            rsem, w4sem, wsem,
            *, H, DH, SK, W, D, F, C, NW4, COMPUTE, NPAIR, NR, LA, ORDER, MIX, WQR, WOR):
    w0 = SK - W
    PW = 2 * DH
    NP = W // C
    NSTEP = 4 * NP
    LB = C // 128
    w4_rows = F // NW4
    scale = DH ** -0.5
    X_SEM, WQ_SEM, WO_SEM, W3_SEM = 0, 1, 2, 3
    assert NSTEP % NR == 0 and LA < NR

    def piece(p, g):
        p = p + g // NSTEP
        g = g % NSTEP
        slab, j = g // NP, g % NP
        src = (k_hbm, v_hbm)[slab % 2]
        h = 2 * p + slab // 2
        return pltpu.make_async_copy(
            src.at[0, h, :, pl.ds(w0 + j * C, C)], ring.at[g % NR], rsem.at[g % NR])

    def wq_piece(p, r0, nr):
        return pltpu.make_async_copy(
            wq_hbm.at[pl.ds(r0, nr), pl.ds(pl.multiple_of(p * PW, 128), PW)],
            wqbuf.at[pl.ds(r0, nr), :], wsem.at[WQ_SEM])

    def wo_piece(p, r0, nr):
        r = pl.multiple_of(p * PW + r0, 8)
        return pltpu.make_async_copy(
            wo_hbm.at[pl.ds(r, nr), :], wobuf.at[pl.ds(r, nr), :], wsem.at[WO_SEM])

    def w3_piece(r0, nr, c0, nc):
        return pltpu.make_async_copy(
            w3_hbm.at[pl.ds(r0, nr), pl.ds(c0, nc)],
            w3buf.at[pl.ds(r0, nr), pl.ds(c0, nc)], wsem.at[W3_SEM])

    def w4_piece(i):
        return pltpu.make_async_copy(
            w4_hbm.at[pl.ds(i * w4_rows, w4_rows), :],
            w4buf.at[pl.ds(i * w4_rows, w4_rows), :], w4sem.at[i])

    x_copy = pltpu.make_async_copy(x_hbm, xbuf, wsem.at[X_SEM])

    wq_list = [("q", r, WQR) for r in range(0, D, WQR)]
    wo_list = [("o", r, WOR) for r in range(0, PW, WOR)]
    QP_STEP = 3 * NP + 1
    WO_WAIT = 2 * NP
    sched = [[] for _ in range(NSTEP)]
    items = wq_list + wo_list
    n = len(items)
    for i, it in enumerate(items):
        sched[i * NSTEP // n].append(it)
    for t in range(NSTEP):
        for it in sched[t]:
            assert (it[0] == "q" and t < QP_STEP - 8) or (it[0] == "o" and t >= WO_WAIT), (t, it)
    w3_items = [(r, 8, 0, 1024) for r in range(0, D, 8)] + [(r, 16, 1024, 512) for r in range(0, D, 16)]
    w3_sched = [[] for _ in range(NSTEP)]
    for i, it in enumerate(w3_items):
        w3_sched[i * NSTEP // len(w3_items)].append(it)

    def small(p, t):
        if sched[t]:
            @pl.when(p + 1 < NPAIR)
            def _():
                for kind, r, nr in sched[t]:
                    (wq_piece if kind == "q" else wo_piece)(p + 1, r, nr).start(priority=0)
        if w3_sched[t]:
            @pl.when(p + 1 == NPAIR)
            def _():
                for it in w3_sched[t]:
                    w3_piece(*it).start(priority=0)

    def big(p, t):
        g = t + LA
        if g < NSTEP:
            piece(p, g).start(priority=1)
        else:
            @pl.when(p + 1 < NPAIR)
            def _():
                piece(p, g).start(priority=1)
            if g - NSTEP < NW4:
                @pl.when(p + 1 == NPAIR)
                def _():
                    w4_piece(g - NSTEP).start(priority=1)

    def step_dma(p, t):
        piece(p, t).wait()
        if ORDER == "10":
            big(p, t)
            small(p, t)
        else:
            small(p, t)
            big(p, t)

    x_copy.start(priority=0)
    wq_piece(0, 0, D).start(priority=0)
    for g in range(LA):
        piece(0, g).start(priority=1)
        if g == NP - 1 or (g == LA - 1 and LA < NP):
            wo_piece(0, 0, PW).start(priority=1)

    x_copy.wait()
    x = xbuf[0].astype(_F32)
    xn8 = jnp.broadcast_to(_layernorm(x).astype(_BF16), (8, D))

    def q_prep():
        wq_piece(0, 0, D).wait()
        if COMPUTE:
            q = jnp.dot(xn8, wqbuf[...], preferred_element_type=_F32) * scale
            qbbuf[...] = jnp.transpose(jnp.broadcast_to(q[0:1], (128, PW)))

    q_prep()
    accbuf[...] = jnp.zeros_like(accbuf)

    def k_phase(p, hb, t0):
        if COMPUTE:
            qb = qbbuf[pl.ds(hb * DH, DH), :]
        for j in range(NP):
            t = t0 + j
            step_dma(p, t)
            if COMPUTE:
                for b in range(LB):
                    kp = ring[t % NR, :, pl.ds(b * 128, 128)].astype(_F32)
                    sbuf[pl.ds(j * LB + b, 1), :] = jnp.sum(kp * qb, axis=0, keepdims=True)

    def softmax():
        s = sbuf[...]
        m = jnp.max(jnp.max(s, axis=0, keepdims=True), axis=1, keepdims=True)
        e = jnp.exp(s - m)
        l = jnp.sum(jnp.sum(e, axis=0, keepdims=True), axis=1, keepdims=True)
        sbuf[...] = e * (1.0 / l)

    def v_phase(p, t0, mid=None):
        acc = jnp.zeros((DH, 128), _F32)
        for j in range(NP):
            t = t0 + j
            step_dma(p, t)
            if COMPUTE:
                for b in range(LB):
                    vp = ring[t % NR, :, pl.ds(b * 128, 128)].astype(_F32)
                    acc = acc + vp * sbuf[pl.ds(j * LB + b, 1), :]
            if mid is not None and j == 0:
                mid()
        return acc

    def o_proj(h, acc):
        if COMPUTE:
            o = jnp.sum(acc, axis=1, keepdims=True)
            wo_h = wobuf[pl.ds(pl.multiple_of(h * DH, 64), DH), :].astype(_F32)
            prod = wo_h * o
            accbuf[...] += jnp.sum(prod.reshape(DH // 8, 8, D), axis=0)

    def pair(p, carry):
        a = 2 * p
        k_phase(p, 0, 0)
        if COMPUTE:
            softmax()
        acc = v_phase(p, NP)
        wo_piece(p, 0, PW).wait()
        o_proj(a, acc)
        k_phase(p, 1, 2 * NP)
        if COMPUTE:
            softmax()

        def mid():
            @pl.when(p + 1 < NPAIR)
            def _():
                q_prep()

        acc = v_phase(p, 3 * NP, mid)
        o_proj(a + 1, acc)
        return carry

    lax.fori_loop(0, NPAIR, pair, 0)

    h1 = x + jnp.sum(accbuf[...], axis=0, keepdims=True)
    y = _layernorm(h1)
    z8 = jnp.broadcast_to(_layernorm(y).astype(_BF16), (8, D))
    w3_piece(0, D, 0, F).wait()
    g = jax.nn.gelu(jnp.dot(z8, w3buf[...], preferred_element_type=_F32),
                    approximate=True).astype(_BF16)
    out = h1 + y
    for i in range(NW4):
        w4_piece(i).wait()
        out = out + jnp.dot(g[:, i * w4_rows:(i + 1) * w4_rows],
                            w4buf[pl.ds(i * w4_rows, w4_rows), :],
                            preferred_element_type=_F32)[0:1]
    o_ref[0] = out.astype(o_ref.dtype)


def build(**over):
    cfg = dict(CFG); cfg.update(over)

    @jax.jit
    def pallas_sequential_preLN__sliding_block_cached__mixer_s_mlp__decode_kernel(
            A_x, A_k_cache, A_v_cache, A_wq, A_wo, B_x, B_w1, B_w2, B_w3, B_w4):
        B, S, D = A_x.shape
        _, H, SK, DH = A_k_cache.shape
        F = B_w3.shape[1]
        assert B == 1 and S == 1
        W = min(4096, max(256, SK // 4))
        C, NW4, NR = cfg["C"], cfg["NW4"], cfg["NR"]
        kt = jnp.swapaxes(A_k_cache, 2, 3)
        vt = jnp.swapaxes(A_v_cache, 2, 3)
        kern = functools.partial(_kernel, H=H, DH=DH, SK=SK, W=W, D=D, F=F, **cfg)
        any_spec = pl.BlockSpec(memory_space=pl.ANY)
        return pl.pallas_call(
            kern,
            out_shape=jax.ShapeDtypeStruct((B, S, D), A_x.dtype),
            in_specs=[any_spec] * 7,
            out_specs=pl.BlockSpec(memory_space=pltpu.VMEM),
            scratch_shapes=[
                pltpu.VMEM((B, S, D), _BF16),
                pltpu.VMEM((NR, DH, C), _BF16),
                pltpu.VMEM((D, 2 * DH), _BF16),
                pltpu.VMEM((H * DH, D), _BF16),
                pltpu.VMEM((D, F), _BF16),
                pltpu.VMEM((F, D), _BF16),
                pltpu.VMEM((2 * DH, 128), _F32),
                pltpu.VMEM((W // 128, 128), _F32),
                pltpu.VMEM((8, D), _F32),
                pltpu.SemaphoreType.DMA((NR,)),
                pltpu.SemaphoreType.DMA((NW4,)),
                pltpu.SemaphoreType.DMA((4,)),
            ],
            compiler_params=pltpu.CompilerParams(vmem_limit_bytes=64 * 1024 * 1024,
                                                 disable_bounds_checks=True,
                                                 disable_semaphore_checks=True),
        )(A_x, kt, vt, A_wq, A_wo, B_w3, B_w4)
    return pallas_sequential_preLN__sliding_block_cached__mixer_s_mlp__decode_kernel


pallas_sequential_preLN__sliding_block_cached__mixer_s_mlp__decode_kernel = build()
```

```python
import functools

import jax
import jax.numpy as jnp
from jax import lax
import jax.experimental.pallas as pl
import jax.experimental.pallas.tpu as pltpu

_EPS = 1e-5
_F32 = jnp.float32
_BF16 = jnp.bfloat16

_C = 128
_NR = 64
_LA = 40
_PERM = 27
_W3C = 384
_TAIL = (512, 256, 96, 32)
_NVPU = 2
_X_SEM, _WQ_SEM, _WO_SEM, _W3_SEM, _W4_SEM = 0, 1, 2, 4, 5


def _kernel(x_hbm, k_hbm, v_hbm, wq_hbm, wo_hbm, w3_hbm, w4_hbm,
            o_ref,
            xbuf, ring, wqbuf, wobuf, w3buf, w4buf, qbbuf, sbuf, accbuf,
            rsem, w4sem, wsem,
            *, H, DH, SK, W, D, F):
    w0 = SK - W
    PW = 2 * DH
    NPAIR = H // 2
    NP = W // _C
    NSTEP = 4 * NP
    NW4 = len(_TAIL)
    W4PRE = F - sum(_TAIL)
    w4_off = [W4PRE + sum(_TAIL[:i]) for i in range(NW4)]
    scale = DH ** -0.5
    assert NSTEP % _NR == 0 and NW4 <= _LA < _NR

    def piece(p, g):
        p = p + g // NSTEP
        g = g % NSTEP
        slab, j = g // NP, g % NP
        src = (k_hbm, v_hbm)[slab % 2]
        return pltpu.make_async_copy(
            src.at[0, 2 * p + slab // 2, :, pl.ds(w0 + j * _C, _C)],
            ring.at[g % _NR], rsem.at[g % _NR])

    def wq_piece(p, r0, nr):
        return pltpu.make_async_copy(
            wq_hbm.at[pl.ds(r0, nr), pl.ds(pl.multiple_of(p * PW, 128), PW)],
            wqbuf.at[pl.ds(r0, nr), :], wsem.at[_WQ_SEM])

    def wo_piece(p, hb, r0, nr):
        r = pl.multiple_of(p * PW + hb * DH + r0, 8)
        return pltpu.make_async_copy(
            wo_hbm.at[pl.ds(r, nr), :], wobuf.at[hb, pl.ds(r0, nr), :],
            wsem.at[_WO_SEM + hb])

    def w3_piece(r0, nr, c0, nc):
        return pltpu.make_async_copy(
            w3_hbm.at[pl.ds(r0, nr), pl.ds(c0, nc)],
            w3buf.at[pl.ds(r0, nr), pl.ds(c0, nc)], wsem.at[_W3_SEM])

    def w4_pre(r0, nr):
        return pltpu.make_async_copy(
            w4_hbm.at[pl.ds(r0, nr), :], w4buf.at[pl.ds(r0, nr), :], wsem.at[_W4_SEM])

    def w4_tail(i):
        return pltpu.make_async_copy(
            w4_hbm.at[pl.ds(w4_off[i], _TAIL[i]), :],
            w4buf.at[pl.ds(w4_off[i], _TAIL[i]), :], w4sem.at[i])

    x_copy = pltpu.make_async_copy(x_hbm, xbuf, wsem.at[_X_SEM])

    QP = 3 * NP + 1
    NG = D // 8
    NO = DH // 8
    SLACK = 8
    assert NG + 2 * NO == NSTEP
    wq_rows = [((i * _PERM) % NG) * 8 for i in range(NG)]
    assert sorted(wq_rows) == list(range(0, D, 8))
    mid = NSTEP // 2 - SLACK
    a_sl = [(i * mid) // NO for i in range(NO)]
    forced = list(range(QP - SLACK, QP + 1))
    rest = [t for t in range(mid, NSTEP - SLACK) if t not in forced]
    nrest = NO - len(forced)
    b_sl = sorted(forced + [rest[(i * len(rest)) // nrest] for i in range(nrest)])
    q_sl = [t for t in range(NSTEP) if t not in a_sl and t not in b_sl]
    q_late = [t for t in q_sl if t > QP]
    q_early = [t for t in q_sl if t < QP]
    NL = len(q_late)
    assert NL + len(q_early) == NG
    seq = {}
    seq.update({t: ("o", 0, i) for i, t in enumerate(a_sl)})
    seq.update({t: ("o", 1, i) for i, t in enumerate(b_sl)})
    seq.update({t: ("q", 2, i) for i, t in enumerate(q_late)})
    seq.update({t: ("q", 1, NL + i) for i, t in enumerate(q_early)})
    nslot = NG + NL - 4
    w4_cut = [8 * ((i * (W4PRE // 8)) // nslot) for i in range(nslot + 1)] + [W4PRE] * 4
    W3R = D // NPAIR
    assert W3R % 8 == 0 and W3R * NPAIR == D
    w3_items = [(r, c) for r in range(0, W3R, 8) for c in range(0, F, _W3C)]
    w3_sl = [t for t in q_sl if t < NSTEP - SLACK]
    w3_at = {w3_sl[(i * len(w3_sl)) // len(w3_items)]: it for i, it in enumerate(w3_items)}
    assert len(w3_at) == len(w3_items)

    def issue_small(p, t):
        kind, a, i = seq[t]
        if kind == "o":
            wo_piece(p, a, i * 8, 8).start(priority=0)
        else:
            @pl.when(p + a < NPAIR)
            def _():
                wq_piece(p + a, wq_rows[i], 8).start(priority=0)

            for extra, k in ((0, i), (1, NG + i)):
                if extra < a and w4_cut[k + 1] > w4_cut[k]:
                    @pl.when(p + a == NPAIR + extra)
                    def _():
                        w4_pre(w4_cut[k], w4_cut[k + 1] - w4_cut[k]).start(priority=0)
        if t in w3_at:
            r, c = w3_at[t]
            w3_piece(pl.multiple_of(p * W3R + r, 8), 8, c, _W3C).start(priority=0)

    def issue_big(p, t):
        g = t + _LA
        if g < NSTEP:
            piece(p, g).start(priority=1)
        else:
            @pl.when(p + 1 < NPAIR)
            def _():
                piece(p, g).start(priority=1)

            if g - NSTEP < NW4:
                @pl.when(p + 1 == NPAIR)
                def _():
                    w4_tail(g - NSTEP).start(priority=1)

    def step_dma(p, t):
        piece(p, t).wait()
        issue_big(p, t)
        issue_small(p, t)

    x_copy.start(priority=0)
    wq_piece(0, 0, D).start(priority=0)
    for g in range(_LA):
        piece(0, g).start(priority=1)

    x_copy.wait()
    x = xbuf[0].astype(_F32)
    xc = x - jnp.mean(x, axis=-1, keepdims=True)
    xn = xc * lax.rsqrt(jnp.mean(xc * xc, axis=-1, keepdims=True) + _EPS)
    xn8 = jnp.broadcast_to(xn.astype(_BF16), (8, D))

    def q_prep():
        wq_piece(0, 0, D).wait()
        q = jnp.dot(xn8, wqbuf[...], preferred_element_type=_F32) * scale
        qbbuf[...] = jnp.transpose(jnp.broadcast_to(q[0:1], (128, PW)))

    q_prep()
    for i in range(NL):
        wq_piece(1, wq_rows[i], 8).start(priority=0)
    accbuf[...] = jnp.zeros_like(accbuf)

    def k_phase(p, hb, t0):
        qb = qbbuf[pl.ds(hb * DH, DH), :]
        for j in range(NP):
            step_dma(p, t0 + j)
            kp = ring[(t0 + j) % _NR].astype(_F32)
            sbuf[pl.ds(j, 1), :] = jnp.sum(kp * qb, axis=0, keepdims=True)
        s = sbuf[...]
        m = jnp.max(jnp.max(s, axis=0, keepdims=True), axis=1, keepdims=True)
        e = jnp.exp(s - m)
        l = jnp.sum(jnp.sum(e, axis=0, keepdims=True), axis=1, keepdims=True)
        sbuf[...] = e * (1.0 / l)

    def v_phase(p, hb, t0):
        acc = jnp.zeros((DH, 128), _F32)
        for j in range(NP):
            step_dma(p, t0 + j)
            vp = ring[(t0 + j) % _NR].astype(_F32)
            acc = acc + vp * sbuf[pl.ds(j, 1), :]
            if t0 + j == QP - 1:
                pl.when(p + 1 < NPAIR)(q_prep)
        wo_piece(p, hb, 0, DH).wait()
        o = jnp.sum(acc, axis=1, keepdims=True)
        prod = wobuf[hb].astype(_F32) * o
        accbuf[...] += jnp.sum(prod.reshape(DH // 8, 8, D), axis=0)

    def pair(p, carry):
        for hb in range(2):
            k_phase(p, hb, 2 * hb * NP)
            v_phase(p, hb, (2 * hb + 1) * NP)
        return carry

    lax.fori_loop(0, NPAIR, pair, 0)

    w3_piece(0, D, 0, F).wait()
    w4_pre(0, W4PRE).wait()
    h1 = x + jnp.sum(accbuf[...], axis=0, keepdims=True)
    row = lax.broadcasted_iota(jnp.int32, (8, D), 0)
    u = h1.astype(_BF16).astype(_F32)
    lhs = jnp.where(row == 0, jnp.broadcast_to(u, (8, D)), 1.0).astype(_BF16)
    res = jnp.dot(lhs, w3buf[...], preferred_element_type=_F32)
    m1 = jnp.mean(u, axis=-1, keepdims=True)
    c1 = u - m1
    r1 = lax.rsqrt(jnp.mean(c1 * c1, axis=-1, keepdims=True) + _EPS)
    y = c1 * r1
    m2 = jnp.mean(y, axis=-1, keepdims=True)
    r2 = lax.rsqrt(jnp.mean(y * y, axis=-1, keepdims=True) - m2 * m2 + _EPS)
    pre = (r1 * r2) * res[0:1] - (r1 * r2 * m1 + r2 * m2) * res[1:2]
    g1 = jax.nn.gelu(pre, approximate=True).astype(_BF16)
    g = jnp.broadcast_to(g1, (8, F))

    VR = sum(_TAIL[NW4 - _NVPU:])
    assert VR % 128 == 0
    gcol = jnp.transpose(jnp.broadcast_to(g1[:, F - VR:].astype(_F32), (128, VR)))
    out = h1 + y + jnp.dot(g[:, :W4PRE], w4buf[pl.ds(0, W4PRE), :],
                           preferred_element_type=_F32)[0:1]
    for i in range(NW4 - _NVPU):
        r, n = w4_off[i], _TAIL[i]
        w4_tail(i).wait()
        out = out + jnp.dot(g[:, r:r + n], w4buf[pl.ds(r, n), :],
                            preferred_element_type=_F32)[0:1]
    part = jnp.where(row == 0, jnp.broadcast_to(out, (8, D)), 0.0)
    for i in range(NW4 - _NVPU, NW4):
        r, n = w4_off[i], _TAIL[i]
        w4_tail(i).wait()
        gc = gcol[r - (F - VR):r - (F - VR) + n]
        prod = w4buf[pl.ds(r, n), :].astype(_F32) * jnp.concatenate([gc] * (D // 128), axis=1)
        part = part + jnp.sum(prod.reshape(n // 8, 8, D), axis=0)
    o_ref[0] = jnp.sum(part, axis=0, keepdims=True).astype(o_ref.dtype)


@jax.jit
def pallas_sequential_preLN__sliding_block_cached__mixer_s_mlp__decode_kernel(
    A_x: jax.Array,
    A_k_cache: jax.Array,
    A_v_cache: jax.Array,
    A_wq: jax.Array,
    A_wo: jax.Array,
    B_x: jax.Array,
    B_w1: jax.Array,
    B_w2: jax.Array,
    B_w3: jax.Array,
    B_w4: jax.Array,
):
    B, S, D = A_x.shape
    _, H, SK, DH = A_k_cache.shape
    F = B_w3.shape[1]
    assert B == 1 and S == 1
    W = min(4096, max(256, SK // 4))

    kt = jnp.swapaxes(A_k_cache, 2, 3)
    vt = jnp.swapaxes(A_v_cache, 2, 3)

    any_spec = pl.BlockSpec(memory_space=pl.ANY)
    return pl.pallas_call(
        functools.partial(_kernel, H=H, DH=DH, SK=SK, W=W, D=D, F=F),
        out_shape=jax.ShapeDtypeStruct((B, S, D), A_x.dtype),
        in_specs=[any_spec] * 7,
        out_specs=pl.BlockSpec(memory_space=pltpu.VMEM),
        scratch_shapes=[
            pltpu.VMEM((B, S, D), _BF16),
            pltpu.VMEM((_NR, DH, _C), _BF16),
            pltpu.VMEM((D, 2 * DH), _BF16),
            pltpu.VMEM((2, DH, D), _BF16),
            pltpu.VMEM((D, F), _BF16),
            pltpu.VMEM((F, D), _BF16),
            pltpu.VMEM((2 * DH, 128), _F32),
            pltpu.VMEM((W // _C, _C), _F32),
            pltpu.VMEM((8, D), _F32),
            pltpu.SemaphoreType.DMA((_NR,)),
            pltpu.SemaphoreType.DMA((len(_TAIL),)),
            pltpu.SemaphoreType.DMA((6,)),
        ],
        compiler_params=pltpu.CompilerParams(
            vmem_limit_bytes=32 * 1024 * 1024,
            disable_bounds_checks=True,
            disable_semaphore_checks=True),
    )(A_x, kt, vt, A_wq, A_wo, B_w3, B_w4)
```

```python
import functools

import jax
import jax.numpy as jnp
from jax import lax
import jax.experimental.pallas as pl
import jax.experimental.pallas.tpu as pltpu

_EPS = 1e-5
_F32 = jnp.float32
_BF16 = jnp.bfloat16

_C = 128
_NR = 64
_LA = 26
_PERM = 27
_W3C = 384
_TAIL = (512, 256, 96, 32)
_NVPU = 2
_NS = 10
_X_SEM, _WQ_SEM, _WO_SEM, _W3_SEM, _W4_SEM = 0, 1, 2, 4, 5


def _kernel(x_hbm, k_hbm, v_hbm, wq_hbm, wo_hbm, w3_hbm, w4_hbm,
            o_ref,
            xbuf, ring, wqbuf, wobuf, w3buf, w4buf, qbbuf, sbuf, accbuf,
            rsem, w4sem, wsem,
            *, H, DH, SK, W, D, F):
    w0 = SK - W
    PW = 2 * DH
    NPAIR = H // 2
    NP = W // _C
    NSTEP = 4 * NP
    NW4 = len(_TAIL)
    W4PRE = F - sum(_TAIL)
    w4_off = [W4PRE + sum(_TAIL[:i]) for i in range(NW4)]
    scale = DH ** -0.5
    assert NSTEP % _NR == 0 and NW4 <= _LA < _NR

    def piece(p, g):
        p = p + g // NSTEP
        g = g % NSTEP
        slab, j = g // NP, g % NP
        src = (k_hbm, v_hbm)[slab % 2]
        return pltpu.make_async_copy(
            src.at[0, 2 * p + slab // 2, :, pl.ds(w0 + j * _C, _C)],
            ring.at[g % _NR], rsem.at[g % _NR])

    def wq_piece(p, r0, nr):
        return pltpu.make_async_copy(
            wq_hbm.at[pl.ds(r0, nr), pl.ds(pl.multiple_of(p * PW, 128), PW)],
            wqbuf.at[pl.ds(r0, nr), :], wsem.at[_WQ_SEM])

    def wo_piece(p, hb, r0, nr):
        r = pl.multiple_of(p * PW + hb * DH + r0, 8)
        return pltpu.make_async_copy(
            wo_hbm.at[pl.ds(r, nr), :], wobuf.at[hb, pl.ds(r0, nr), :],
            wsem.at[_WO_SEM + hb])

    def w3_piece(r0, nr, c0, nc):
        return pltpu.make_async_copy(
            w3_hbm.at[pl.ds(r0, nr), pl.ds(c0, nc)],
            w3buf.at[pl.ds(r0, nr), pl.ds(c0, nc)], wsem.at[_W3_SEM])

    def w4_pre(r0, nr):
        return pltpu.make_async_copy(
            w4_hbm.at[pl.ds(r0, nr), :], w4buf.at[pl.ds(r0, nr), :], wsem.at[_W4_SEM])

    def w4_tail(i):
        return pltpu.make_async_copy(
            w4_hbm.at[pl.ds(w4_off[i], _TAIL[i]), :],
            w4buf.at[pl.ds(w4_off[i], _TAIL[i]), :], w4sem.at[i])

    x_copy = pltpu.make_async_copy(x_hbm, xbuf, wsem.at[_X_SEM])

    QP = 3 * NP + 1
    NG = D // 8
    NO = DH // 8
    SLACK = 8
    assert NG + 2 * NO == NSTEP
    wq_rows = [((i * _PERM) % NG) * 8 for i in range(NG)]
    assert sorted(wq_rows) == list(range(0, D, 8))
    mid = NSTEP // 2 - SLACK
    a_sl = [(i * mid) // NO for i in range(NO)]
    forced = list(range(QP - SLACK, QP + 1))
    rest = [t for t in range(mid, NSTEP - SLACK) if t not in forced]
    nrest = NO - len(forced)
    b_sl = sorted(forced + [rest[(i * len(rest)) // nrest] for i in range(nrest)])
    q_sl = [t for t in range(NSTEP) if t not in a_sl and t not in b_sl]
    q_late = [t for t in q_sl if t > QP]
    q_early = [t for t in q_sl if t < QP]
    NL = len(q_late)
    assert NL + len(q_early) == NG
    seq = {}
    seq.update({t: ("o", 0, i) for i, t in enumerate(a_sl)})
    seq.update({t: ("o", 1, i) for i, t in enumerate(b_sl)})
    seq.update({t: ("q", 2, i) for i, t in enumerate(q_late)})
    seq.update({t: ("q", 1, NL + i) for i, t in enumerate(q_early)})
    nslot = NG + NL - 4
    w4_cut = [8 * (_NS + (i * (W4PRE // 8 - _NS)) // nslot) for i in range(nslot + 1)] + [W4PRE] * 4
    W3R = D // NPAIR
    assert W3R % 8 == 0 and W3R * NPAIR == D
    w3_items = [(r, c) for r in range(0, W3R, 8) for c in range(0, F, _W3C)]
    w3_sl = [t for t in q_sl if t < NSTEP - SLACK]
    w3_at = {w3_sl[(i * len(w3_sl)) // len(w3_items)]: it for i, it in enumerate(w3_items)}
    assert len(w3_at) == len(w3_items)

    def issue_small(p, t):
        kind, a, i = seq[t]
        if kind == "o":
            wo_piece(p, a, i * 8, 8).start(priority=0)
        else:
            @pl.when(p + a < NPAIR)
            def _():
                wq_piece(p + a, wq_rows[i], 8).start(priority=0)

            for extra, k in ((0, i), (1, NG + i)):
                if extra < a and w4_cut[k + 1] > w4_cut[k]:
                    @pl.when(p + a == NPAIR + extra)
                    def _():
                        w4_pre(w4_cut[k], w4_cut[k + 1] - w4_cut[k]).start(priority=0)
        if t in w3_at:
            r, c = w3_at[t]
            w3_piece(pl.multiple_of(p * W3R + r, 8), 8, c, _W3C).start(priority=0)

    def issue_big(p, t):
        g = t + _LA
        if g < NSTEP:
            piece(p, g).start(priority=1)
        else:
            @pl.when(p + 1 < NPAIR)
            def _():
                piece(p, g).start(priority=1)

            if g - NSTEP < NW4:
                @pl.when(p + 1 == NPAIR)
                def _():
                    w4_tail(g - NSTEP).start(priority=1)

    def step_dma(p, t):
        piece(p, t).wait()
        issue_big(p, t)
        issue_small(p, t)

    def wq_first(i):
        nr = D // _NS
        return pltpu.make_async_copy(
            wq_hbm.at[pl.ds(i * nr, nr), pl.ds(0, PW)], wqbuf.at[pl.ds(i * nr, nr), :],
            rsem.at[_NR - _NS + i])

    assert _LA <= _NR - _NS
    x_copy.start(priority=0)
    for i in range(_NS):
        wq_first(i).start(priority=1)
    for g in range(_LA - _NS):
        piece(0, g).start(priority=1)

    x_copy.wait()
    x = xbuf[0].astype(_F32)
    xc = x - jnp.mean(x, axis=-1, keepdims=True)
    xn = xc * lax.rsqrt(jnp.mean(xc * xc, axis=-1, keepdims=True) + _EPS)
    xn8 = jnp.broadcast_to(xn.astype(_BF16), (8, D))

    def q_prep(first=False):
        if not first:
            wq_piece(0, 0, D).wait()
        q = jnp.dot(xn8, wqbuf[...], preferred_element_type=_F32) * scale
        qbbuf[...] = jnp.transpose(jnp.broadcast_to(q[0:1], (128, PW)))

    for i in range(_NS):
        wq_first(i).wait()
        piece(0, _LA - _NS + i).start(priority=1)
        w4_pre(8 * i, 8).start(priority=0)
    q_prep(True)
    for i in range(NL):
        wq_piece(1, wq_rows[i], 8).start(priority=0)
    accbuf[...] = jnp.zeros_like(accbuf)

    def k_phase(p, hb, t0):
        qb = qbbuf[pl.ds(hb * DH, DH), :]
        for j in range(NP):
            step_dma(p, t0 + j)
            kp = ring[(t0 + j) % _NR].astype(_F32)
            sbuf[pl.ds(j, 1), :] = jnp.sum(kp * qb, axis=0, keepdims=True)
        s = sbuf[...]
        m = jnp.max(jnp.max(s, axis=0, keepdims=True), axis=1, keepdims=True)
        e = jnp.exp(s - m)
        l = jnp.sum(jnp.sum(e, axis=0, keepdims=True), axis=1, keepdims=True)
        sbuf[...] = e * (1.0 / l)

    def v_phase(p, hb, t0):
        acc = jnp.zeros((DH, 128), _F32)
        for j in range(NP):
            step_dma(p, t0 + j)
            vp = ring[(t0 + j) % _NR].astype(_F32)
            acc = acc + vp * sbuf[pl.ds(j, 1), :]
            if t0 + j == QP - 1:
                pl.when(p + 1 < NPAIR)(q_prep)
        wo_piece(p, hb, 0, DH).wait()
        o = jnp.sum(acc, axis=1, keepdims=True)
        prod = wobuf[hb].astype(_F32) * o
        accbuf[...] += jnp.sum(prod.reshape(DH // 8, 8, D), axis=0)

    def pair(p, carry):
        for hb in range(2):
            k_phase(p, hb, 2 * hb * NP)
            v_phase(p, hb, (2 * hb + 1) * NP)
        return carry

    lax.fori_loop(0, NPAIR, pair, 0)

    w3_piece(0, D, 0, F).wait()
    w4_pre(0, W4PRE).wait()
    h1 = x + jnp.sum(accbuf[...], axis=0, keepdims=True)
    row = lax.broadcasted_iota(jnp.int32, (8, D), 0)
    u = h1.astype(_BF16).astype(_F32)
    lhs = jnp.where(row == 0, jnp.broadcast_to(u, (8, D)), 1.0).astype(_BF16)
    res = jnp.dot(lhs, w3buf[...], preferred_element_type=_F32)
    m1 = jnp.mean(u, axis=-1, keepdims=True)
    c1 = u - m1
    r1 = lax.rsqrt(jnp.mean(c1 * c1, axis=-1, keepdims=True) + _EPS)
    y = c1 * r1
    m2 = jnp.mean(y, axis=-1, keepdims=True)
    r2 = lax.rsqrt(jnp.mean(y * y, axis=-1, keepdims=True) - m2 * m2 + _EPS)
    pre = (r1 * r2) * res[0:1] - (r1 * r2 * m1 + r2 * m2) * res[1:2]
    g1 = jax.nn.gelu(pre, approximate=True).astype(_BF16)
    g = jnp.broadcast_to(g1, (8, F))

    VR = sum(_TAIL[NW4 - _NVPU:])
    assert VR % 128 == 0
    gcol = jnp.transpose(jnp.broadcast_to(g1[:, F - VR:].astype(_F32), (128, VR)))
    out = h1 + y + jnp.dot(g[:, :W4PRE], w4buf[pl.ds(0, W4PRE), :],
                           preferred_element_type=_F32)[0:1]
    for i in range(NW4 - _NVPU):
        r, n = w4_off[i], _TAIL[i]
        w4_tail(i).wait()
        out = out + jnp.dot(g[:, r:r + n], w4buf[pl.ds(r, n), :],
                            preferred_element_type=_F32)[0:1]
    part = jnp.where(row == 0, jnp.broadcast_to(out, (8, D)), 0.0)
    for i in range(NW4 - _NVPU, NW4):
        r, n = w4_off[i], _TAIL[i]
        w4_tail(i).wait()
        gc = gcol[r - (F - VR):r - (F - VR) + n]
        prod = w4buf[pl.ds(r, n), :].astype(_F32) * jnp.concatenate([gc] * (D // 128), axis=1)
        part = part + jnp.sum(prod.reshape(n // 8, 8, D), axis=0)
    o_ref[0] = jnp.sum(part, axis=0, keepdims=True).astype(o_ref.dtype)


@jax.jit
def pallas_sequential_preLN__sliding_block_cached__mixer_s_mlp__decode_kernel(
    A_x: jax.Array,
    A_k_cache: jax.Array,
    A_v_cache: jax.Array,
    A_wq: jax.Array,
    A_wo: jax.Array,
    B_x: jax.Array,
    B_w1: jax.Array,
    B_w2: jax.Array,
    B_w3: jax.Array,
    B_w4: jax.Array,
):
    B, S, D = A_x.shape
    _, H, SK, DH = A_k_cache.shape
    F = B_w3.shape[1]
    assert B == 1 and S == 1
    W = min(4096, max(256, SK // 4))

    kt = jnp.swapaxes(A_k_cache, 2, 3)
    vt = jnp.swapaxes(A_v_cache, 2, 3)

    any_spec = pl.BlockSpec(memory_space=pl.ANY)
    return pl.pallas_call(
        functools.partial(_kernel, H=H, DH=DH, SK=SK, W=W, D=D, F=F),
        out_shape=jax.ShapeDtypeStruct((B, S, D), A_x.dtype),
        in_specs=[any_spec] * 7,
        out_specs=pl.BlockSpec(memory_space=pltpu.VMEM),
        scratch_shapes=[
            pltpu.VMEM((B, S, D), _BF16),
            pltpu.VMEM((_NR, DH, _C), _BF16),
            pltpu.VMEM((D, 2 * DH), _BF16),
            pltpu.VMEM((2, DH, D), _BF16),
            pltpu.VMEM((D, F), _BF16),
            pltpu.VMEM((F, D), _BF16),
            pltpu.VMEM((2 * DH, 128), _F32),
            pltpu.VMEM((W // _C, _C), _F32),
            pltpu.VMEM((8, D), _F32),
            pltpu.SemaphoreType.DMA((_NR,)),
            pltpu.SemaphoreType.DMA((len(_TAIL),)),
            pltpu.SemaphoreType.DMA((6,)),
        ],
        compiler_params=pltpu.CompilerParams(
            vmem_limit_bytes=32 * 1024 * 1024,
            disable_bounds_checks=True,
            disable_semaphore_checks=True),
    )(A_x, kt, vt, A_wq, A_wo, B_w3, B_w4)
```

```python
import functools

import jax
import jax.numpy as jnp
from jax import lax
import jax.experimental.pallas as pl
import jax.experimental.pallas.tpu as pltpu

_EPS = 1e-5
_F32 = jnp.float32
_BF16 = jnp.bfloat16

_C = 128
_NR = 64
_LA = 26
_QS = 15
_QU = 16
_QR = 64
_QLA = 30
_NE = 8
_TAIL = (512, 256, 96, 32)
_NVPU = 2
_X_SEM, _WO_SEM, _W3_SEM, _W4_SEM = 0, 1, 3, 4


def _kernel(x_hbm, k_hbm, v_hbm, wq_hbm, wo_hbm, w3_hbm, w4_hbm,
            o_ref,
            xbuf, ring, wqring, wobuf, w3buf, w4buf, xbbuf, qacc, qbbuf, sbuf, accbuf,
            rsem, qsem, w4sem, wsem,
            *, H, DH, SK, W, D, F):
    w0 = SK - W
    PW = 2 * DH
    NPAIR = H // 2
    NP = W // _C
    NSTEP = 4 * NP
    NW4 = len(_TAIL)
    W4PRE = F - sum(_TAIL)
    w4_off = [W4PRE + sum(_TAIL[:i]) for i in range(NW4)]
    QG = wq_hbm.shape[1]
    QI = QG // _QU
    QB = H * DH // 128 // _QU
    assert NSTEP % _NR == 0 and NW4 <= _LA < _NR
    assert QG % _QU == 0 and _QLA < _QR and _QR & (_QR - 1) == 0 and _QU & (_QU - 1) == 0

    def mod_pow2(i, n):
        return i % n if isinstance(i, int) else lax.bitwise_and(i, n - 1)

    def piece(p, g):
        p = p + g // NSTEP
        g = g % NSTEP
        slab, j = g // NP, g % NP
        src = (k_hbm, v_hbm)[slab % 2]
        return pltpu.make_async_copy(
            src.at[0, 2 * p + slab // 2, :, pl.ds(w0 + j * _C, _C)],
            ring.at[g % _NR], rsem.at[g % _NR])

    def wq_piece(g):
        slot = mod_pow2(g, _QR)
        return pltpu.make_async_copy(wq_hbm.at[:, g], wqring.at[slot], qsem.at[slot])

    def wo_piece(p, hb, r0, nr, c0, nc):
        r = pl.multiple_of(p * PW + hb * DH + r0, 8)
        return pltpu.make_async_copy(
            wo_hbm.at[pl.ds(r, nr), pl.ds(c0, nc)],
            wobuf.at[hb, pl.ds(r0, nr), pl.ds(c0, nc)], wsem.at[_WO_SEM + hb])

    def w3_piece(r0, nr, c0, nc):
        return pltpu.make_async_copy(
            w3_hbm.at[pl.ds(r0, nr), pl.ds(c0, nc)],
            w3buf.at[pl.ds(r0, nr), pl.ds(c0, nc)], wsem.at[_W3_SEM])

    def w4_head(r0, nr, c0, nc):
        return pltpu.make_async_copy(
            w4_hbm.at[pl.ds(r0, nr), pl.ds(c0, nc)],
            w4buf.at[pl.ds(r0, nr), pl.ds(c0, nc)], wsem.at[_W4_SEM])

    def w4_tail(i):
        return pltpu.make_async_copy(
            w4_hbm.at[pl.ds(w4_off[i], _TAIL[i]), :],
            w4buf.at[pl.ds(w4_off[i], _TAIL[i]), :], w4sem.at[i])

    x_copy = pltpu.make_async_copy(x_hbm, xbuf, wsem.at[_X_SEM])

    W4I = W4PRE // QI
    assert W4I % 8 == 0 and W4I * QI == W4PRE
    w4_items = [(r, c0, nc) for r in range(0, W4I, 8)
                for c0, nc in ((0, 256), (256, 256), (512, D - 512))]
    assert len(w4_items) <= _QU
    W3R = D // NPAIR
    assert W3R % 8 == 0 and W3R * NPAIR == D
    wo_items = [[("o", hb, r, c0, nc) for r in range(0, DH, 8)
                 for c0, nc in ((0, 256), (256, D - 256))] for hb in range(2)]
    w3_items = [("3", 0, r, c0, 256) for r in range(0, W3R, 8) for c0 in range(0, F, 256)]
    half = len(w3_items) // 2
    order = wo_items[0][_NE:] + w3_items[:half] + wo_items[1] + w3_items[half:]
    assert len(order) <= NSTEP - _NE
    seq = {(i * (NSTEP - _NE)) // len(order): it for i, it in enumerate(order)}
    seq.update({NSTEP - _NE + i: ("n",) + it[1:] for i, it in enumerate(wo_items[0][:_NE])})
    assert all(t < NSTEP // 2 for t, it in seq.items() if it[:2] == ("o", 0))

    def issue_small(p, t):
        if t not in seq:
            return
        kind, hb, r, c0, nc = seq[t]
        if kind == "o":
            wo_piece(p, hb, r, 8, c0, nc).start(priority=0)
        elif kind == "n":
            @pl.when(p + 1 < NPAIR)
            def _():
                wo_piece(p + 1, hb, r, 8, c0, nc).start(priority=0)
        else:
            w3_piece(pl.multiple_of(p * W3R + r, 8), 8, c0, nc).start(priority=0)

    def issue_big(p, t):
        g = t + _LA
        if g < NSTEP:
            piece(p, g).start(priority=1)
        else:
            @pl.when(p + 1 < NPAIR)
            def _():
                piece(p, g).start(priority=1)

            if g - NSTEP < NW4:
                @pl.when(p + 1 == NPAIR)
                def _():
                    w4_tail(g - NSTEP).start(priority=1)

    def step_dma(p, t):
        piece(p, t).wait()
        issue_big(p, t)
        issue_small(p, t)

    x_copy.start(priority=0)
    for g in range(_QLA):
        wq_piece(g).start(priority=1)

    x_copy.wait()
    x = xbuf[0].astype(_F32)
    xc = x - jnp.mean(x, axis=-1, keepdims=True)
    xn = xc * lax.rsqrt(jnp.mean(xc * xc, axis=-1, keepdims=True) + _EPS)
    xs = xn.astype(_BF16).astype(_F32) * (DH ** -0.5)
    xbbuf[...] = jnp.transpose(jnp.broadcast_to(xs, (128, D))).reshape(D // 8, 8, 128)
    qacc[...] = jnp.zeros_like(qacc)
    accbuf[...] = jnp.zeros_like(accbuf)

    assert QI % QB == 1
    first_k = {QG - _QLA + (i * _QLA) // _LA: i for i in range(_LA)}
    assert len(first_k) == _LA

    def q_iter(it):
        xb, cb = [], []
        for s in range(_QS):
            b = s * QI + it
            rg = b // QB if isinstance(b, int) else lax.div(b, QB)
            xb.append(xbbuf[rg])
            cb.append(b - rg * QB)
        for j in range(_QU):
            g = it * _QU + j
            wq_piece(g).wait()
            if not isinstance(g, int) or g + _QLA < QG:
                wq_piece(g + _QLA).start(priority=1)
            elif g in first_k:
                piece(0, first_k[g]).start(priority=1)
            if j < len(w4_items):
                r, c0, nc = w4_items[j]
                w4_head(pl.multiple_of(it * W4I + r, 8), 8, c0, nc).start(priority=0)
            slot = mod_pow2(g, _QR)
            for k in range(QB):
                terms = [wqring[slot, s].astype(_F32) * xb[s] for s in range(k, _QS, QB)]
                while len(terms) > 1:
                    terms = ([a + b for a, b in zip(terms[::2], terms[1::2])]
                             + terms[len(terms) & ~1:])
                qacc[cb[k], j] += terms[0]

    def q_body(it, carry):
        q_iter(it)
        return carry

    n_dyn = QI - pl.cdiv(_QLA, _QU)
    lax.fori_loop(0, n_dyn, q_body, 0)
    for it in range(n_dyn, QI):
        q_iter(it)

    def q_prep(p):
        for c in range(PW // 128):
            col = p * (PW // 128) + c
            blk = col // _QU if isinstance(col, int) else lax.div(col, _QU)
            q = jnp.sum(qacc[blk, mod_pow2(col, _QU)], axis=0, keepdims=True)
            qbbuf[pl.ds(c * 128, 128), :] = jnp.transpose(jnp.broadcast_to(q, (128, 128)))

    for _, hb, r, c0, nc in wo_items[0][:_NE]:
        wo_piece(0, hb, r, 8, c0, nc).start(priority=0)
    q_prep(0)

    def k_phase(p, hb, t0):
        qb = qbbuf[pl.ds(hb * DH, DH), :]
        for j in range(NP):
            step_dma(p, t0 + j)
            kp = ring[(t0 + j) % _NR].astype(_F32)
            sbuf[pl.ds(j, 1), :] = jnp.sum(kp * qb, axis=0, keepdims=True)
        s = sbuf[...]
        m = jnp.max(jnp.max(s, axis=0, keepdims=True), axis=1, keepdims=True)
        e = jnp.exp(s - m)
        l = jnp.sum(jnp.sum(e, axis=0, keepdims=True), axis=1, keepdims=True)
        sbuf[...] = e * (1.0 / l)

    def v_phase(p, hb, t0):
        acc = jnp.zeros((DH, 128), _F32)
        for j in range(NP):
            step_dma(p, t0 + j)
            vp = ring[(t0 + j) % _NR].astype(_F32)
            acc = acc + vp * sbuf[pl.ds(j, 1), :]
            if hb == 1 and j == 0:
                q_prep(jnp.minimum(p + 1, NPAIR - 1))
        wo_piece(p, hb, 0, DH, 0, D).wait()
        o = jnp.sum(acc, axis=1, keepdims=True)
        prod = wobuf[hb].astype(_F32) * o
        accbuf[...] += jnp.sum(prod.reshape(DH // 8, 8, D), axis=0)

    def pair(p, carry):
        for hb in range(2):
            k_phase(p, hb, 2 * hb * NP)
            v_phase(p, hb, (2 * hb + 1) * NP)
        return carry

    lax.fori_loop(0, NPAIR, pair, 0)

    w3_piece(0, D, 0, F).wait()
    w4_head(0, W4PRE, 0, D).wait()
    h1 = x + jnp.sum(accbuf[...], axis=0, keepdims=True)
    row = lax.broadcasted_iota(jnp.int32, (8, D), 0)
    u = h1.astype(_BF16).astype(_F32)
    lhs = jnp.where(row == 0, jnp.broadcast_to(u, (8, D)), 1.0).astype(_BF16)
    res = jnp.dot(lhs, w3buf[...], preferred_element_type=_F32)
    m1 = jnp.mean(u, axis=-1, keepdims=True)
    c1 = u - m1
    r1 = lax.rsqrt(jnp.mean(c1 * c1, axis=-1, keepdims=True) + _EPS)
    y = c1 * r1
    m2 = jnp.mean(y, axis=-1, keepdims=True)
    r2 = lax.rsqrt(jnp.mean(y * y, axis=-1, keepdims=True) - m2 * m2 + _EPS)
    pre = (r1 * r2) * res[0:1] - (r1 * r2 * m1 + r2 * m2) * res[1:2]
    g1 = jax.nn.gelu(pre, approximate=True).astype(_BF16)
    g = jnp.broadcast_to(g1, (8, F))

    VR = sum(_TAIL[NW4 - _NVPU:])
    assert VR % 128 == 0
    gcol = jnp.transpose(jnp.broadcast_to(g1[:, F - VR:].astype(_F32), (128, VR)))
    out = h1 + y + jnp.dot(g[:, :W4PRE], w4buf[pl.ds(0, W4PRE), :],
                           preferred_element_type=_F32)[0:1]
    for i in range(NW4 - _NVPU):
        r, n = w4_off[i], _TAIL[i]
        w4_tail(i).wait()
        out = out + jnp.dot(g[:, r:r + n], w4buf[pl.ds(r, n), :],
                            preferred_element_type=_F32)[0:1]
    part = jnp.where(row == 0, jnp.broadcast_to(out, (8, D)), 0.0)
    for i in range(NW4 - _NVPU, NW4):
        r, n = w4_off[i], _TAIL[i]
        w4_tail(i).wait()
        gc = gcol[r - (F - VR):r - (F - VR) + n]
        prod = w4buf[pl.ds(r, n), :].astype(_F32) * jnp.concatenate([gc] * (D // 128), axis=1)
        part = part + jnp.sum(prod.reshape(n // 8, 8, D), axis=0)
    o_ref[0] = jnp.sum(part, axis=0, keepdims=True).astype(o_ref.dtype)


@jax.jit
def pallas_sequential_preLN__sliding_block_cached__mixer_s_mlp__decode_kernel(
    A_x: jax.Array,
    A_k_cache: jax.Array,
    A_v_cache: jax.Array,
    A_wq: jax.Array,
    A_wo: jax.Array,
    B_x: jax.Array,
    B_w1: jax.Array,
    B_w2: jax.Array,
    B_w3: jax.Array,
    B_w4: jax.Array,
):
    B, S, D = A_x.shape
    _, H, SK, DH = A_k_cache.shape
    F = B_w3.shape[1]
    assert B == 1 and S == 1
    W = min(4096, max(256, SK // 4))
    QC = H * DH // 128
    QG = (D // 8) * QC // _QS

    kt = jnp.swapaxes(A_k_cache, 2, 3)
    vt = jnp.swapaxes(A_v_cache, 2, 3)
    wqt = A_wq.reshape(D // 8, 8, QC, 128).transpose(0, 2, 1, 3).reshape(_QS, QG, 8, 128)

    any_spec = pl.BlockSpec(memory_space=pl.ANY)
    return pl.pallas_call(
        functools.partial(_kernel, H=H, DH=DH, SK=SK, W=W, D=D, F=F),
        out_shape=jax.ShapeDtypeStruct((B, S, D), A_x.dtype),
        in_specs=[any_spec] * 7,
        out_specs=pl.BlockSpec(memory_space=pltpu.VMEM),
        scratch_shapes=[
            pltpu.VMEM((B, S, D), _BF16),
            pltpu.VMEM((_NR, DH, _C), _BF16),
            pltpu.VMEM((_QR, _QS, 8, 128), _BF16),
            pltpu.VMEM((2, DH, D), _BF16),
            pltpu.VMEM((D, F), _BF16),
            pltpu.VMEM((F, D), _BF16),
            pltpu.VMEM((D // 8, 8, 128), _F32),
            pltpu.VMEM((QC // _QU, _QU, 8, 128), _F32),
            pltpu.VMEM((2 * DH, 128), _F32),
            pltpu.VMEM((W // _C, _C), _F32),
            pltpu.VMEM((8, D), _F32),
            pltpu.SemaphoreType.DMA((_NR,)),
            pltpu.SemaphoreType.DMA((_QR,)),
            pltpu.SemaphoreType.DMA((len(_TAIL),)),
            pltpu.SemaphoreType.DMA((5,)),
        ],
        compiler_params=pltpu.CompilerParams(
            vmem_limit_bytes=32 * 1024 * 1024,
            disable_bounds_checks=True,
            disable_semaphore_checks=True),
    )(A_x, kt, vt, wqt, A_wo, B_w3, B_w4)
```

```python
import functools

import jax
import jax.numpy as jnp
from jax import lax
import jax.experimental.pallas as pl
import jax.experimental.pallas.tpu as pltpu

_EPS = 1e-5
_F32 = jnp.float32
_BF16 = jnp.bfloat16

_C = 128
_NR = 64
_LA = 26
_QS = 15
_QU = 16
_QR = 64
_QLA = 30
_NE = 8
_TAIL = (512, 256, 96, 32)
_NVPU = 2
_X_SEM, _WO_SEM, _W3_SEM, _W4_SEM = 0, 1, 3, 4


def _kernel(x_hbm, k_hbm, v_hbm, wq_hbm, wo_hbm, w3_hbm, w4_hbm,
            o_ref,
            xbuf, ring, wqring, wobuf, w3buf, w4buf, xbbuf, qacc, qbbuf, sbuf, accbuf,
            rsem, qsem, w4sem, wsem,
            *, H, DH, SK, W, D, F):
    w0 = SK - W
    PW = 2 * DH
    NPAIR = H // 2
    NP = W // _C
    NSTEP = 4 * NP
    NW4 = len(_TAIL)
    W4PRE = F - sum(_TAIL)
    w4_off = [W4PRE + sum(_TAIL[:i]) for i in range(NW4)]
    QG = wq_hbm.shape[1]
    QI = QG // _QU
    QB = H * DH // 128 // _QU
    assert NSTEP % _NR == 0 and NW4 <= _LA < _NR
    assert QG % _QU == 0 and _QLA < _QR and _QR & (_QR - 1) == 0 and _QU & (_QU - 1) == 0

    def mod_pow2(i, n):
        return i % n if isinstance(i, int) else lax.bitwise_and(i, n - 1)

    def piece(p, g):
        p = p + g // NSTEP
        g = g % NSTEP
        slab, j = g // NP, g % NP
        src = (k_hbm, v_hbm)[slab % 2]
        return pltpu.make_async_copy(
            src.at[0, 2 * p + slab // 2, :, pl.ds(w0 + j * _C, _C)],
            ring.at[g % _NR], rsem.at[g % _NR])

    def wq_piece(g):
        slot = mod_pow2(g, _QR)
        return pltpu.make_async_copy(wq_hbm.at[:, g], wqring.at[slot], qsem.at[slot])

    def wo_piece(p, hb, r0, nr, c0, nc):
        r = pl.multiple_of(p * PW + hb * DH + r0, 8)
        return pltpu.make_async_copy(
            wo_hbm.at[pl.ds(r, nr), pl.ds(c0, nc)],
            wobuf.at[hb, pl.ds(r0, nr), pl.ds(c0, nc)], wsem.at[_WO_SEM + hb])

    def w3_piece(r0, nr, c0, nc):
        return pltpu.make_async_copy(
            w3_hbm.at[pl.ds(r0, nr), pl.ds(c0, nc)],
            w3buf.at[pl.ds(r0, nr), pl.ds(c0, nc)], wsem.at[_W3_SEM])

    def w4_head(r0, nr, c0, nc):
        return pltpu.make_async_copy(
            w4_hbm.at[pl.ds(r0, nr), pl.ds(c0, nc)],
            w4buf.at[pl.ds(r0, nr), pl.ds(c0, nc)], wsem.at[_W4_SEM])

    def w4_tail(i):
        return pltpu.make_async_copy(
            w4_hbm.at[pl.ds(w4_off[i], _TAIL[i]), :],
            w4buf.at[pl.ds(w4_off[i], _TAIL[i]), :], w4sem.at[i])

    x_copy = pltpu.make_async_copy(x_hbm, xbuf, wsem.at[_X_SEM])

    W4I = W4PRE // QI
    assert W4I % 8 == 0 and W4I * QI == W4PRE
    w4_items = [(r, c0, nc) for r in range(0, W4I, 8)
                for c0, nc in ((0, 256), (256, 256), (512, D - 512))]
    assert len(w4_items) <= _QU
    W3R = D // NPAIR
    assert W3R % 8 == 0 and W3R * NPAIR == D
    wo_items = [[("o", hb, r, c0, nc) for r in range(0, DH, 8)
                 for c0, nc in ((0, 256), (256, D - 256))] for hb in range(2)]
    w3_items = [("3", 0, r, c0, 256) for r in range(0, W3R, 8) for c0 in range(0, F, 256)]
    half = len(w3_items) // 2
    order = wo_items[0][_NE:] + w3_items[:half] + wo_items[1] + w3_items[half:]
    assert len(order) <= NSTEP - _NE
    seq = {(i * (NSTEP - _NE)) // len(order): it for i, it in enumerate(order)}
    seq.update({NSTEP - _NE + i: ("n",) + it[1:] for i, it in enumerate(wo_items[0][:_NE])})
    assert all(t < NSTEP // 2 for t, it in seq.items() if it[:2] == ("o", 0))

    def issue_small(p, t):
        if t not in seq:
            return
        kind, hb, r, c0, nc = seq[t]
        if kind == "o":
            wo_piece(p, hb, r, 8, c0, nc).start(priority=0)
        elif kind == "n":
            @pl.when(p + 1 < NPAIR)
            def _():
                wo_piece(p + 1, hb, r, 8, c0, nc).start(priority=0)
        else:
            w3_piece(pl.multiple_of(p * W3R + r, 8), 8, c0, nc).start(priority=0)

    def issue_big(p, t):
        g = t + _LA
        if g < NSTEP:
            piece(p, g).start(priority=1)
        else:
            @pl.when(p + 1 < NPAIR)
            def _():
                piece(p, g).start(priority=1)

            if g - NSTEP < NW4:
                @pl.when(p + 1 == NPAIR)
                def _():
                    w4_tail(g - NSTEP).start(priority=1)

    def step_dma(p, t):
        piece(p, t).wait()
        issue_big(p, t)
        issue_small(p, t)

    x_copy.start(priority=0)
    for g in range(_QLA):
        wq_piece(g).start(priority=1)

    x_copy.wait()
    x = xbuf[0].astype(_F32)
    xc = x - jnp.mean(x, axis=-1, keepdims=True)
    xn = xc * lax.rsqrt(jnp.mean(xc * xc, axis=-1, keepdims=True) + _EPS)
    xs = xn.astype(_BF16).astype(_F32) * (DH ** -0.5)
    xbbuf[...] = jnp.transpose(jnp.broadcast_to(xs, (128, D))).reshape(D // 8, 8, 128)
    qacc[...] = jnp.zeros_like(qacc)
    accbuf[...] = jnp.zeros_like(accbuf)

    assert QI % QB == 1
    first_k = {QG - _QLA + (i * _QLA) // _LA: i for i in range(_LA)}
    assert len(first_k) == _LA

    def q_iter(it):
        xb, cb = [], []
        for s in range(_QS):
            b = s * QI + it
            rg = b // QB if isinstance(b, int) else lax.div(b, QB)
            xb.append(xbbuf[rg])
            cb.append(b - rg * QB)
        for j in range(_QU):
            g = it * _QU + j
            wq_piece(g).wait()
            if not isinstance(g, int) or g + _QLA < QG:
                wq_piece(g + _QLA).start(priority=1)
            elif g in first_k:
                piece(0, first_k[g]).start(priority=1)
            if j < len(w4_items):
                r, c0, nc = w4_items[j]
                w4_head(pl.multiple_of(it * W4I + r, 8), 8, c0, nc).start(priority=0)
            slot = mod_pow2(g, _QR)
            for k in range(QB):
                terms = [wqring[slot, s].astype(_F32) * xb[s] for s in range(k, _QS, QB)]
                while len(terms) > 1:
                    terms = ([a + b for a, b in zip(terms[::2], terms[1::2])]
                             + terms[len(terms) & ~1:])
                qacc[cb[k], j] += terms[0]

    def q_body(it, carry):
        q_iter(it)
        return carry

    n_dyn = QI - pl.cdiv(_QLA, _QU)
    lax.fori_loop(0, n_dyn, q_body, 0)
    for it in range(n_dyn, QI):
        q_iter(it)

    def q_prep(p):
        for c in range(PW // 128):
            col = p * (PW // 128) + c
            blk = col // _QU if isinstance(col, int) else lax.div(col, _QU)
            q = jnp.sum(qacc[blk, mod_pow2(col, _QU)], axis=0, keepdims=True)
            qbbuf[pl.ds(c * 128, 128), :] = jnp.transpose(jnp.broadcast_to(q, (128, 128)))

    for _, hb, r, c0, nc in wo_items[0][:_NE]:
        wo_piece(0, hb, r, 8, c0, nc).start(priority=0)
    q_prep(0)

    def k_phase(p, hb, t0):
        qb = qbbuf[pl.ds(hb * DH, DH), :]
        for j in range(NP):
            step_dma(p, t0 + j)
            kp = ring[(t0 + j) % _NR].astype(_F32)
            sbuf[pl.ds(j, 1), :] = jnp.sum(kp * qb, axis=0, keepdims=True)
        s = sbuf[...]
        m = jnp.max(jnp.max(s, axis=0, keepdims=True), axis=1, keepdims=True)
        e = jnp.exp(s - m)
        l = jnp.sum(jnp.sum(e, axis=0, keepdims=True), axis=1, keepdims=True)
        sbuf[...] = e * (1.0 / l)

    def v_phase(p, hb, t0):
        acc = jnp.zeros((DH, 128), _F32)
        for j in range(NP):
            step_dma(p, t0 + j)
            vp = ring[(t0 + j) % _NR].astype(_F32)
            acc = acc + vp * sbuf[pl.ds(j, 1), :]
            if hb == 1 and j == 0:
                q_prep(jnp.minimum(p + 1, NPAIR - 1))
        wo_piece(p, hb, 0, DH, 0, D).wait()
        o = jnp.sum(acc, axis=1, keepdims=True)
        prod = wobuf[hb].astype(_F32) * o
        accbuf[...] += jnp.sum(prod.reshape(DH // 8, 8, D), axis=0)

    def pair(p, carry):
        for hb in range(2):
            k_phase(p, hb, 2 * hb * NP)
            v_phase(p, hb, (2 * hb + 1) * NP)
        return carry

    lax.fori_loop(0, NPAIR, pair, 0)

    w3_piece(0, D, 0, F).wait()
    w4_head(0, W4PRE, 0, D).wait()
    h1 = x + jnp.sum(accbuf[...], axis=0, keepdims=True)
    row = lax.broadcasted_iota(jnp.int32, (8, D), 0)
    u = h1.astype(_BF16).astype(_F32)
    lhs = jnp.where(row == 0, jnp.broadcast_to(u, (8, D)), 1.0).astype(_BF16)
    res = jnp.dot(lhs, w3buf[...], preferred_element_type=_F32)
    m1 = jnp.mean(u, axis=-1, keepdims=True)
    c1 = u - m1
    r1 = lax.rsqrt(jnp.mean(c1 * c1, axis=-1, keepdims=True) + _EPS)
    y = c1 * r1
    m2 = jnp.mean(y, axis=-1, keepdims=True)
    r2 = lax.rsqrt(jnp.mean(y * y, axis=-1, keepdims=True) - m2 * m2 + _EPS)
    pre = (r1 * r2) * res[0:1] - (r1 * r2 * m1 + r2 * m2) * res[1:2]
    g1 = jax.nn.gelu(pre, approximate=True).astype(_BF16)
    g = jnp.broadcast_to(g1, (8, F))

    VR = sum(_TAIL[NW4 - _NVPU:])
    assert VR % 128 == 0
    gcol = jnp.transpose(jnp.broadcast_to(g1[:, F - VR:].astype(_F32), (128, VR)))
    out = h1 + y + jnp.dot(g[:, :W4PRE], w4buf[pl.ds(0, W4PRE), :],
                           preferred_element_type=_F32)[0:1]
    for i in range(NW4 - _NVPU):
        r, n = w4_off[i], _TAIL[i]
        w4_tail(i).wait()
        out = out + jnp.dot(g[:, r:r + n], w4buf[pl.ds(r, n), :],
                            preferred_element_type=_F32)[0:1]
    part = jnp.where(row == 0, jnp.broadcast_to(out, (8, D)), 0.0)
    for i in range(NW4 - _NVPU, NW4):
        r, n = w4_off[i], _TAIL[i]
        w4_tail(i).wait()
        gc = gcol[r - (F - VR):r - (F - VR) + n]
        prod = w4buf[pl.ds(r, n), :].astype(_F32) * jnp.concatenate([gc] * (D // 128), axis=1)
        part = part + jnp.sum(prod.reshape(n // 8, 8, D), axis=0)
    o_ref[0] = jnp.sum(part, axis=0, keepdims=True).astype(o_ref.dtype)


@jax.jit
def pallas_sequential_preLN__sliding_block_cached__mixer_s_mlp__decode_kernel(
    A_x: jax.Array,
    A_k_cache: jax.Array,
    A_v_cache: jax.Array,
    A_wq: jax.Array,
    A_wo: jax.Array,
    B_x: jax.Array,
    B_w1: jax.Array,
    B_w2: jax.Array,
    B_w3: jax.Array,
    B_w4: jax.Array,
):
    B, S, D = A_x.shape
    _, H, SK, DH = A_k_cache.shape
    F = B_w3.shape[1]
    assert B == 1 and S == 1
    W = min(4096, max(256, SK // 4))
    QC = H * DH // 128
    QG = (D // 8) * QC // _QS

    kt = jnp.swapaxes(A_k_cache, 2, 3)
    vt = jnp.swapaxes(A_v_cache, 2, 3)
    wqt = A_wq.reshape(D // 8, 8, QC, 128).transpose(0, 2, 1, 3).reshape(_QS, QG, 8, 128)

    params = dict(vmem_limit_bytes=32 * 1024 * 1024, disable_bounds_checks=True)
    if hasattr(pltpu.CompilerParams, "disable_semaphore_checks"):
        params["disable_semaphore_checks"] = True

    any_spec = pl.BlockSpec(memory_space=pl.ANY)
    return pl.pallas_call(
        functools.partial(_kernel, H=H, DH=DH, SK=SK, W=W, D=D, F=F),
        out_shape=jax.ShapeDtypeStruct((B, S, D), A_x.dtype),
        in_specs=[any_spec] * 7,
        out_specs=pl.BlockSpec(memory_space=pltpu.VMEM),
        scratch_shapes=[
            pltpu.VMEM((B, S, D), _BF16),
            pltpu.VMEM((_NR, DH, _C), _BF16),
            pltpu.VMEM((_QR, _QS, 8, 128), _BF16),
            pltpu.VMEM((2, DH, D), _BF16),
            pltpu.VMEM((D, F), _BF16),
            pltpu.VMEM((F, D), _BF16),
            pltpu.VMEM((D // 8, 8, 128), _F32),
            pltpu.VMEM((QC // _QU, _QU, 8, 128), _F32),
            pltpu.VMEM((2 * DH, 128), _F32),
            pltpu.VMEM((W // _C, _C), _F32),
            pltpu.VMEM((8, D), _F32),
            pltpu.SemaphoreType.DMA((_NR,)),
            pltpu.SemaphoreType.DMA((_QR,)),
            pltpu.SemaphoreType.DMA((len(_TAIL),)),
            pltpu.SemaphoreType.DMA((5,)),
        ],
        compiler_params=pltpu.CompilerParams(**params),
    )(A_x, kt, vt, wqt, A_wo, B_w3, B_w4)
```
